```python
import jax
import jax.numpy as jnp

def _softmax(x, axis=-1):
    return jax.nn.softmax(x, axis=axis)
def _gelu(x):
    return jax.nn.gelu(x, approximate=True)
def _silu(x):
    return jax.nn.silu(x)
def _sigmoid(x):
    return jax.nn.sigmoid(x)
def _layernorm(x, axis=-1, eps=1e-5):
    m = jnp.mean(x, axis=axis, keepdims=True)
    v = jnp.var(x, axis=axis, keepdims=True)
    return (x - m) / jnp.sqrt(v + eps)
def _scatter_add(tgt, idx, src, axis=0):
    return tgt.at[idx].add(src)
def _segment_sum(src, seg, n):
    return jax.ops.segment_sum(src, seg, n)
class _Rng:
    def __init__(self, key):
        self._k = key
    def _next(self):
        self._k, sub = jax.random.split(self._k)
        return sub
    def normal(self, shape):
        return jax.random.normal(self._next(), shape, dtype=jnp.bfloat16)
    def randint(self, lo, hi, shape):
        return jax.random.randint(self._next(), shape, lo, hi, dtype=jnp.int32)
    def uniform(self, shape, lo=0.0, hi=1.0):
        return jax.random.uniform(self._next(), shape, jnp.bfloat16, lo, hi)
    def permutation(self, n):
        return jax.random.permutation(self._next(), n)


kernel_name = 'recurrent_scan__sliding_block_cached__mixer_s_mlp__decode'

def setup_inputs():
    _rng = _Rng(jax.random.key(int.from_bytes(__import__("os").urandom(4), "little")))
    _w = (lambda a: (lambda t: t.astype(jnp.bfloat16) if jnp.issubdtype(t.dtype, jnp.floating) else t)(jnp.asarray(a)))
    def _A_setup():
        B, Sq, D = 1, 1, 512
        Hq, Hkv, Sk, Dh = 32, 32, 32768, 128
        assert Hq % Hkv == 0, (Hq, Hkv)
        return {
            "x": _w((lambda *s: _rng.normal(s) * 0.05)(B, Sq, D)),
            "k_cache": _w((lambda *s: _rng.normal(s) * 0.05)(B, Hkv, Sk, Dh)),
            "v_cache": _w((lambda *s: _rng.normal(s) * 0.05)(B, Hkv, Sk, Dh)),
            "wq": _w((lambda *s: _rng.normal(s) * 0.05)(D, Hq * Dh) * (D ** -0.5)),
            "wo": _w((lambda *s: _rng.normal(s) * 0.05)(Hq * Dh, D) * ((Hq * Dh) ** -0.5)),
        }
    _A_in = _A_setup()

    def _B_setup():
        B, S, D, F = 1, 1, 512, 1376
        return {
            "x":  _w((lambda *s: _rng.normal(s) * 0.05)(B, S, D)),
            "w1": _w((lambda *s: _rng.normal(s) * 0.05)(D, D) * (D ** -0.5)),
            "w2": _w((lambda *s: _rng.normal(s) * 0.05)(D, D) * (D ** -0.5)),
            "w3": _w((lambda *s: _rng.normal(s) * 0.05)(D, F) * (D ** -0.5)),
            "w4": _w((lambda *s: _rng.normal(s) * 0.05)(F, D) * (F ** -0.5)),
        }
    _B_in = _B_setup()

    return {
        "A_x": _A_in["x"],
        "A_k_cache": _A_in["k_cache"],
        "A_v_cache": _A_in["v_cache"],
        "A_wq": _A_in["wq"],
        "A_wo": _A_in["wo"],
        "B_x": _B_in["x"],
        "B_w1": _B_in["w1"],
        "B_w2": _B_in["w2"],
        "B_w3": _B_in["w3"],
        "B_w4": _B_in["w4"],
    }

def reference(A_x, A_k_cache, A_v_cache, A_wq, A_wo, B_x, B_w1, B_w2, B_w3, B_w4):
    def _A_ref(x, k_cache, v_cache, wq, wo):
        B, Sq, D = x.shape
        Hq, Dh = 32, 128
        Hkv, Sk = k_cache.shape[1], k_cache.shape[2]
        W = min(4096, max(256, Sk // 4))
        rep = Hq // Hkv
        q = (lambda x, *d: x.transpose(*d))((x @ wq).reshape(B, Sq, Hq, Dh), 0, 2, 1, 3)
        k = jnp.repeat(k_cache[:, :, Sk - W:, :], rep, axis=1)
        v = jnp.repeat(v_cache[:, :, Sk - W:, :], rep, axis=1)
        scores = jnp.einsum("bhqd,bhkd->bhqk", q, k) * (Dh ** -0.5)
        p = _softmax(scores, axis=-1)
        o = jnp.einsum("bhqk,bhkd->bhqd", p, v)
        return (lambda x, *d: x.transpose(*d))(o, 0, 2, 1, 3).reshape(B, Sq, Hq * Dh) @ wo

    def _B_ref(x, w1, w2, w3, w4):
        B, S, D = x.shape
        h = _gelu(_layernorm(x, axis=-1) @ w1)
        c = D // 4
        g0 = jnp.pad(h[:, :, 0*c:1*c], ((0, 0), (1, 0), (0, 0)))[:, :S, :]
        g1 = jnp.pad(h[:, :, 1*c:2*c], ((0, 0), (0, 1), (0, 0)))[:, 1:, :]
        g2 = jnp.pad(h[:, :, 2*c:3*c], ((0, 0), (2, 0), (0, 0)))[:, :S, :]
        g3 = jnp.pad(h[:, :, 3*c:   ], ((0, 0), (0, 2), (0, 0)))[:, 2:, :]
        hs = jnp.concatenate([g0, g1, g2, g3], axis=-1) @ w2
        x1 = x + hs
        h2 = _gelu(_layernorm(x1, axis=-1) @ w3) @ w4
        return x1 + h2

    x = A_x
    xn = _layernorm(x, axis=-1)
    s = _A_ref(xn, A_k_cache, A_v_cache, A_wq, A_wo)
    g = _silu(_B_ref(xn, B_w1, B_w2, B_w3, B_w4))
    return x + s * g
```

```python
import jax
import jax.numpy as jnp
from jax import lax
import jax.experimental.pallas as pl
import jax.experimental.pallas.tpu as pltpu

_H, _DH = 32, 128
_KV_CHUNKS = (16, 12, 4)
_WO_CHUNKS = (16, 8, 6, 2)
_DEPTH = 6
_NT = (((1,), (1,)), ((), ()))
_F32, _BF16 = jnp.float32, jnp.bfloat16


def _layernorm(x):
    d = x - jnp.mean(x, axis=-1, keepdims=True)
    v = jnp.mean(d * d, axis=-1, keepdims=True)
    return d / jnp.sqrt(v + 1e-5)


def _kernel(x_hbm, k_hbm, v_hbm, wq_hbm, wo_hbm, w3t_hbm, w4_hbm, o_ref,
            xb, kb, vb, wqb, wob, w3b, w4b, qb, ob, sems):
    sk, w = k_hbm.shape[2], kb.shape[1]
    d = x_hbm.shape[-1]

    copies = []

    def add(src, dst):
        copies.append(pltpu.make_async_copy(src, dst, sems.at[len(copies)]))

    add(wq_hbm, wqb)
    add(x_hbm, xb)
    r = 0
    for n in _KV_CHUNKS:
        for src, dst in ((k_hbm, kb), (v_hbm, vb)):
            add(src.at[0, pl.ds(r, n), pl.ds(sk - w, w), :], dst.at[pl.ds(r, n)])
        r += n
    add(w3t_hbm, w3b)
    add(w4_hbm, w4b)
    r = 0
    for n in _WO_CHUNKS:
        rows = pl.ds(r * _DH, n * _DH)
        add(wo_hbm.at[rows], wob.at[rows])
        r += n

    for c in copies[:_DEPTH]:
        c.start()
    pending = list(range(len(copies)))

    def wait_next():
        i = pending.pop(0)
        copies[i].wait()
        if i + _DEPTH < len(copies):
            copies[i + _DEPTH].start()

    wait_next()
    wait_next()
    x = xb[0].astype(_F32)
    xn = _layernorm(x).astype(_BF16)
    q = jnp.dot(jnp.broadcast_to(xn, (8, d)), wqb[...],
                preferred_element_type=_F32).astype(_BF16)
    for h in range(_H):
        qb[h] = q[:, h * _DH:(h + 1) * _DH].astype(_F32)

    def head(h, carry):
        s = lax.dot_general(qb[h].astype(_BF16), kb[h], _NT,
                            preferred_element_type=_F32) * (_DH ** -0.5)
        p = jnp.exp(s - jnp.max(s, axis=-1, keepdims=True))
        l = jnp.sum(p, axis=-1, keepdims=True)
        o = jnp.dot(p.astype(_BF16), vb[h], preferred_element_type=_F32)
        ob[h] = o / l
        return carry

    r = 0
    for n in _KV_CHUNKS:
        wait_next()
        wait_next()
        lax.fori_loop(r, r + n, head, 0)
        r += n

    wait_next()
    x1 = xn.astype(_F32)
    hn = jnp.broadcast_to(_layernorm(x1).astype(_BF16), (8, d))
    h1 = lax.dot_general(hn, w3b[...], _NT, preferred_element_type=_F32)
    h1 = jax.nn.gelu(h1, approximate=True).astype(_BF16)
    wait_next()
    h2 = jnp.dot(h1, w4b[...], preferred_element_type=_F32)
    g = jax.nn.silu(x1 + h2[0:1])

    acc = jnp.zeros((8, d), _F32)
    r = 0
    for n in _WO_CHUNKS:
        o = jnp.concatenate([ob[r + j] for j in range(n)], axis=-1).astype(_BF16)
        wait_next()
        acc += jnp.dot(o, wob[r * _DH:(r + n) * _DH, :], preferred_element_type=_F32)
        r += n
    o_ref[0] = (x + acc[0:1] * g).astype(o_ref.dtype)


@jax.jit
def pallas_recurrent_scan__sliding_block_cached__mixer_s_mlp__decode_kernel(
    A_x: jax.Array,
    A_k_cache: jax.Array,
    A_v_cache: jax.Array,
    A_wq: jax.Array,
    A_wo: jax.Array,
    B_x: jax.Array,
    B_w1: jax.Array,
    B_w2: jax.Array,
    B_w3: jax.Array,
    B_w4: jax.Array,
):
    assert A_x.shape[:2] == (1, 1) and A_k_cache.shape[1] == _H
    assert sum(_KV_CHUNKS) == _H and sum(_WO_CHUNKS) == _H
    w = min(4096, max(256, A_k_cache.shape[2] // 4))
    w3t = B_w3.T
    n_copies = 4 + 2 * len(_KV_CHUNKS) + len(_WO_CHUNKS)
    return pl.pallas_call(
        _kernel,
        out_shape=jax.ShapeDtypeStruct(A_x.shape, A_x.dtype),
        in_specs=[pl.BlockSpec(memory_space=pltpu.HBM)] * 7,
        out_specs=pl.BlockSpec(memory_space=pltpu.VMEM),
        scratch_shapes=[
            pltpu.VMEM(A_x.shape, A_x.dtype),
            pltpu.VMEM((_H, w, _DH), A_k_cache.dtype),
            pltpu.VMEM((_H, w, _DH), A_v_cache.dtype),
            pltpu.VMEM(A_wq.shape, A_wq.dtype),
            pltpu.VMEM(A_wo.shape, A_wo.dtype),
            pltpu.VMEM(w3t.shape, w3t.dtype),
            pltpu.VMEM(B_w4.shape, B_w4.dtype),
            pltpu.VMEM((_H, 8, _DH), _F32),
            pltpu.VMEM((_H, 8, _DH), _F32),
            pltpu.SemaphoreType.DMA((n_copies,)),
        ],
        compiler_params=pltpu.CompilerParams(vmem_limit_bytes=100 * 2**20),
    )(A_x, A_k_cache, A_v_cache, A_wq, A_wo, w3t, B_w4)
```

```python
import jax
import jax.numpy as jnp
from jax import lax
import jax.experimental.pallas as pl
import jax.experimental.pallas.tpu as pltpu

_H, _DH = 32, 128
_KV_CHUNKS = (20, 8, 4)
_WO_CHUNKS = (16, 8, 6, 2)
_DEPTH = 6
_NT = (((1,), (1,)), ((), ()))
_F32, _BF16 = jnp.float32, jnp.bfloat16


def _layernorm(x):
    d = x - jnp.mean(x, axis=-1, keepdims=True)
    v = jnp.mean(d * d, axis=-1, keepdims=True)
    return d / jnp.sqrt(v + 1e-5)


def _kernel(x_hbm, k_hbm, v_hbm, wq_hbm, wo_hbm, w3t_hbm, w4_hbm, o_ref,
            xb, kb, vb, wqb, wob, w3b, w4b, qb, ob, sems):
    sk, w = k_hbm.shape[2], kb.shape[1]
    d = x_hbm.shape[-1]

    copies = []

    def add(src, dst):
        copies.append(pltpu.make_async_copy(src, dst, sems.at[len(copies)]))

    add(wq_hbm, wqb)
    add(x_hbm, xb)
    r = 0
    for n in _KV_CHUNKS:
        for src, dst in ((k_hbm, kb), (v_hbm, vb)):
            add(src.at[0, pl.ds(r, n), pl.ds(sk - w, w), :], dst.at[pl.ds(r, n)])
        r += n
    add(w3t_hbm, w3b)
    add(w4_hbm, w4b)
    r = 0
    for n in _WO_CHUNKS:
        rows = pl.ds(r * _DH, n * _DH)
        add(wo_hbm.at[rows], wob.at[rows])
        r += n

    for c in copies[:_DEPTH]:
        c.start()
    pending = list(range(len(copies)))

    def wait_next():
        i = pending.pop(0)
        copies[i].wait()
        if i + _DEPTH < len(copies):
            copies[i + _DEPTH].start()

    wait_next()
    wait_next()
    x = xb[0].astype(_F32)
    xn = _layernorm(x).astype(_BF16)
    q = jnp.dot(jnp.broadcast_to(xn, (8, d)), wqb[...],
                preferred_element_type=_F32).astype(_BF16)
    for h in range(_H):
        qb[h] = q[:, h * _DH:(h + 1) * _DH].astype(_F32)

    def head(h, carry):
        s = lax.dot_general(qb[h].astype(_BF16), kb[h], _NT,
                            preferred_element_type=_F32) * (_DH ** -0.5)
        p = jnp.exp(s - jnp.max(s, axis=-1, keepdims=True))
        l = jnp.sum(p, axis=-1, keepdims=True)
        o = jnp.dot(p.astype(_BF16), vb[h], preferred_element_type=_F32)
        ob[h] = o / l
        return carry

    r = 0
    for n in _KV_CHUNKS:
        wait_next()
        wait_next()
        lax.fori_loop(r, r + n, head, 0)
        r += n

    wait_next()
    x1 = xn.astype(_F32)
    hn = jnp.broadcast_to(_layernorm(x1).astype(_BF16), (8, d))
    h1 = lax.dot_general(hn, w3b[...], _NT, preferred_element_type=_F32)
    h1 = jax.nn.gelu(h1, approximate=True).astype(_BF16)
    wait_next()
    h2 = jnp.dot(h1, w4b[...], preferred_element_type=_F32)
    g = jax.nn.silu(x1 + h2[0:1])

    acc = jnp.zeros((8, d), _F32)
    r = 0
    for n in _WO_CHUNKS:
        o = jnp.concatenate([ob[r + j] for j in range(n)], axis=-1).astype(_BF16)
        wait_next()
        acc += jnp.dot(o, wob[r * _DH:(r + n) * _DH, :], preferred_element_type=_F32)
        r += n
    o_ref[0] = (x + acc[0:1] * g).astype(o_ref.dtype)


@jax.jit
def pallas_recurrent_scan__sliding_block_cached__mixer_s_mlp__decode_kernel(
    A_x: jax.Array,
    A_k_cache: jax.Array,
    A_v_cache: jax.Array,
    A_wq: jax.Array,
    A_wo: jax.Array,
    B_x: jax.Array,
    B_w1: jax.Array,
    B_w2: jax.Array,
    B_w3: jax.Array,
    B_w4: jax.Array,
):
    assert A_x.shape[:2] == (1, 1) and A_k_cache.shape[1] == _H
    assert sum(_KV_CHUNKS) == _H and sum(_WO_CHUNKS) == _H
    w = min(4096, max(256, A_k_cache.shape[2] // 4))
    w3t = B_w3.T
    n_copies = 4 + 2 * len(_KV_CHUNKS) + len(_WO_CHUNKS)
    return pl.pallas_call(
        _kernel,
        out_shape=jax.ShapeDtypeStruct(A_x.shape, A_x.dtype),
        in_specs=[pl.BlockSpec(memory_space=pltpu.HBM)] * 7,
        out_specs=pl.BlockSpec(memory_space=pltpu.VMEM),
        scratch_shapes=[
            pltpu.VMEM(A_x.shape, A_x.dtype),
            pltpu.VMEM((_H, w, _DH), A_k_cache.dtype),
            pltpu.VMEM((_H, w, _DH), A_v_cache.dtype),
            pltpu.VMEM(A_wq.shape, A_wq.dtype),
            pltpu.VMEM(A_wo.shape, A_wo.dtype),
            pltpu.VMEM(w3t.shape, w3t.dtype),
            pltpu.VMEM(B_w4.shape, B_w4.dtype),
            pltpu.VMEM((_H, 8, _DH), _F32),
            pltpu.VMEM((_H, 8, _DH), _F32),
            pltpu.SemaphoreType.DMA((n_copies,)),
        ],
        compiler_params=pltpu.CompilerParams(
            vmem_limit_bytes=100 * 2**20,
            disable_bounds_checks=True,
            disable_semaphore_checks=True,
        ),
    )(A_x, A_k_cache, A_v_cache, A_wq, A_wo, w3t, B_w4)
```
